```python
import jax
import jax.numpy as jnp

def _softmax(x, axis=-1):
    return jax.nn.softmax(x, axis=axis)

def _gelu(x):
    return jax.nn.gelu(x, approximate=True)

def _silu(x):
    return jax.nn.silu(x)

def _sigmoid(x):
    return jax.nn.sigmoid(x)

def _layernorm(x, axis=-1, eps=1e-05):
    m = jnp.mean(x, axis=axis, keepdims=True)
    v = jnp.var(x, axis=axis, keepdims=True)
    return (x - m) / jnp.sqrt(v + eps)

def _scatter_add(tgt, idx, src, axis=0):
    return tgt.at[idx].add(src)

def _segment_sum(src, seg, n):
    return jax.ops.segment_sum(src, seg, n)

class _Rng:

    def __init__(self, key):
        self._k = key

    def _next(self):
        self._k, sub = jax.random.split(self._k)
        return sub

    def normal(self, shape):
        return jax.random.normal(self._next(), shape, dtype=jnp.bfloat16)

    def randint(self, lo, hi, shape):
        return jax.random.randint(self._next(), shape, lo, hi, dtype=jnp.int32)

    def uniform(self, shape, lo=0.0, hi=1.0):
        return jax.random.uniform(self._next(), shape, jnp.bfloat16, lo, hi)

    def permutation(self, n):
        return jax.random.permutation(self._next(), n)
kernel_name = 'adaLN_cond__sliding_block_cached__geglu_ffn__decode'

def setup_inputs():
    _rng = _Rng(jax.random.key(int.from_bytes(__import__("os").urandom(4), "little")))
    _w = lambda a: (lambda t: t.astype(jnp.bfloat16) if jnp.issubdtype(t.dtype, jnp.floating) else t)(jnp.asarray(a))

    def _A_setup():
        B, Sq, D = (1, 1, 640)
        Hq, Hkv, Sk, Dh = (32, 32, 32768, 192)
        assert Hq % Hkv == 0, (Hq, Hkv)
        return {'x': _w((lambda *s: _rng.normal(s) * 0.05)(B, Sq, D)), 'k_cache': _w((lambda *s: _rng.normal(s) * 0.05)(B, Hkv, Sk, Dh)), 'v_cache': _w((lambda *s: _rng.normal(s) * 0.05)(B, Hkv, Sk, Dh)), 'wq': _w((lambda *s: _rng.normal(s) * 0.05)(D, Hq * Dh) * D ** (-0.5)), 'wo': _w((lambda *s: _rng.normal(s) * 0.05)(Hq * Dh, D) * (Hq * Dh) ** (-0.5))}
    _A_in = _A_setup()

    def _B_setup():
        B, S, D, F = (1, 1, 640, 1536)
        return {'x': _w((lambda *s: _rng.normal(s) * 0.05)(B, S, D)), 'w_gate': _w((lambda *s: _rng.normal(s) * 0.05)(D, F)), 'w_up': _w((lambda *s: _rng.normal(s) * 0.05)(D, F)), 'w_down': _w((lambda *s: _rng.normal(s) * 0.05)(F, D))}
    _B_in = _B_setup()
    return {'A_x': _A_in['x'], 'A_k_cache': _A_in['k_cache'], 'A_v_cache': _A_in['v_cache'], 'A_wq': _A_in['wq'], 'A_wo': _A_in['wo'], 'B_x': _B_in['x'], 'B_w_gate': _B_in['w_gate'], 'B_w_up': _B_in['w_up'], 'B_w_down': _B_in['w_down'], 'c': _w((lambda *s: _rng.normal(s) * 0.05)(1, 640)), 'w_mod': _w((lambda *s: _rng.normal(s) * 0.05)(640, 6 * 640) * 640 ** (-0.5))}

def reference(A_x, A_k_cache, A_v_cache, A_wq, A_wo, B_x, B_w_gate, B_w_up, B_w_down, c, w_mod):

    def _A_ref(x, k_cache, v_cache, wq, wo):
        B, Sq, D = x.shape
        Hq, Dh = (32, 192)
        Hkv, Sk = (k_cache.shape[1], k_cache.shape[2])
        W = min(4096, max(256, Sk // 4))
        rep = Hq // Hkv
        q = (lambda x, *d: x.transpose(*d))((x @ wq).reshape(B, Sq, Hq, Dh), 0, 2, 1, 3)
        k = jnp.repeat(k_cache[:, :, Sk - W:, :], rep, axis=1)
        v = jnp.repeat(v_cache[:, :, Sk - W:, :], rep, axis=1)
        scores = jnp.einsum('bhqd,bhkd->bhqk', q, k) * Dh ** (-0.5)
        p = _softmax(scores, axis=-1)
        o = jnp.einsum('bhqk,bhkd->bhqd', p, v)
        return (lambda x, *d: x.transpose(*d))(o, 0, 2, 1, 3).reshape(B, Sq, Hq * Dh) @ wo

    def _B_ref(x, w_gate, w_up, w_down):
        return _gelu(x @ w_gate) * (x @ w_up) @ w_down
    x = A_x
    mod = (_silu(c) @ w_mod).reshape(c.shape[0], 6, 1, -1)
    sa, ca, ga, sb, cb, gb = (mod[:, 0].copy(), mod[:, 1].copy(), mod[:, 2].copy(), mod[:, 3].copy(), mod[:, 4].copy(), mod[:, 5].copy())
    h = _layernorm(x, axis=-1) * (1 + ca) + sa
    x = x + ga * _A_ref(h, A_k_cache, A_v_cache, A_wq, A_wo)
    h = _layernorm(x, axis=-1) * (1 + cb) + sb
    x = x + gb * _B_ref(h, B_w_gate, B_w_up, B_w_down)
    return x
```

```python
import functools
import math

import jax
import jax.numpy as jnp
import jax.experimental.pallas as pl
import jax.experimental.pallas.tpu as pltpu


_H = 32
_DH = 192
_PAIR = 2 * _DH
_NP = _H // 2
_NS = 4
_R = 8
_EPS = 1e-5
_LOG2E = math.log2(math.e)

_NT = (((1,), (1,)), ((), ()))


def _layernorm(x):
    m = jnp.mean(x, axis=-1, keepdims=True)
    d = x - m
    v = jnp.mean(d * d, axis=-1, keepdims=True)
    return d * jax.lax.rsqrt(v + _EPS)


def _dot(a, b):
    return jnp.dot(a, b, preferred_element_type=jnp.float32)


def _kernel(x_hbm, c_hbm, k_hbm, v_hbm, wq_hbm, wo_hbm, wg_hbm, wu_hbm, wd_hbm, wm_hbm,
            o_ref,
            x_buf, c_buf, wm_buf, wq_buf, wo_buf, wg_buf, wu_buf, wd_buf, k_buf, v_buf, q_scr,
            w_sem, kv_sem, *, window, d_model):
    f32, bf16 = jnp.float32, jnp.bfloat16
    sk = k_hbm.shape[1]
    D = d_model

    def kv_copy(src, buf, which, p, slot):
        rows = pl.ds(pl.multiple_of(p * _PAIR, _PAIR), _PAIR)
        return pltpu.make_async_copy(
            src.at[rows, pl.ds(sk - window, window)], buf.at[slot], kv_sem.at[which, slot])

    def kv_start(p, slot):
        kv_copy(k_hbm, k_buf, 0, p, slot).start()
        kv_copy(v_hbm, v_buf, 1, p, slot).start()

    c_cp = pltpu.make_async_copy(c_hbm, c_buf, w_sem.at[0])
    x_cp = pltpu.make_async_copy(x_hbm, x_buf, w_sem.at[1])
    wm_cp = pltpu.make_async_copy(wm_hbm, wm_buf, w_sem.at[2])
    wq_cp = pltpu.make_async_copy(wq_hbm, wq_buf, w_sem.at[3])
    wo_cp = pltpu.make_async_copy(wo_hbm, wo_buf, w_sem.at[4])
    wg_cp = pltpu.make_async_copy(wg_hbm, wg_buf, w_sem.at[5])
    wu_cp = pltpu.make_async_copy(wu_hbm, wu_buf, w_sem.at[6])
    wd_cp = pltpu.make_async_copy(wd_hbm, wd_buf, w_sem.at[7])

    c_cp.start()
    x_cp.start()
    wm_cp.start()
    wq_cp.start()
    wo_cp.start()
    for p in range(_NS):
        kv_start(p, p)

    c_cp.wait()
    c = jnp.broadcast_to(c_buf[...].astype(f32), (_R, D))
    silu_c = (c * jax.nn.sigmoid(c)).astype(bf16)
    wm_cp.wait()
    mod = _dot(silu_c, wm_buf[...])
    sa, ca, ga, sb, cb, gb = (mod[:, i * D:(i + 1) * D] for i in range(6))

    x_cp.wait()
    x = jnp.broadcast_to(x_buf[0].astype(f32), (_R, D))
    h = (_layernorm(x) * (1.0 + ca) + sa).astype(bf16)
    wq_cp.wait()
    row = jax.lax.broadcasted_iota(jnp.int32, (_R, _PAIR), 0)
    col = jax.lax.broadcasted_iota(jnp.int32, (_R, _PAIR), 1)
    diag = (col >= row * _DH) & (col < (row + 1) * _DH)
    for p in range(_NP):
        q = _dot(h, wq_buf[:, p * _PAIR:(p + 1) * _PAIR])
        q_scr[p] = jnp.where(diag, q, 0.0).astype(bf16)

    scale_log2 = (_DH ** -0.5) * _LOG2E
    wo_cp.wait()

    def pair_step(p, acc):
        slot = p % _NS
        kv_copy(k_hbm, k_buf, 0, p, slot).wait()
        s = _dot(q_scr[p], k_buf[slot])
        m = jnp.max(s, axis=-1, keepdims=True)
        e = jnp.exp2((s - m) * scale_log2)
        l = jnp.sum(e, axis=-1, keepdims=True)
        kv_copy(v_hbm, v_buf, 1, p, slot).wait()
        o = jax.lax.dot_general(e.astype(bf16), v_buf[slot], _NT, preferred_element_type=f32)
        o = jnp.where(diag, o / l, 0.0).astype(bf16)

        @pl.when(p + _NS < _NP)
        def _():
            kv_start(p + _NS, slot)

        @pl.when(p + _NS == _NP - 1)
        def _():
            wg_cp.start()
            wu_cp.start()
            wd_cp.start()

        return acc + _dot(o, wo_buf[p])

    attn = jax.lax.fori_loop(0, _NP, pair_step, jnp.zeros((_R, D), f32))
    attn = jnp.sum(attn, axis=0, keepdims=True)
    x1 = x + ga * attn

    h2 = (_layernorm(x1) * (1.0 + cb) + sb).astype(bf16)
    wg_cp.wait()
    g = _dot(h2, wg_buf[...])
    wu_cp.wait()
    u = _dot(h2, wu_buf[...])
    a = (jax.nn.gelu(g, approximate=True) * u).astype(bf16)
    wd_cp.wait()
    y = _dot(a, wd_buf[...])
    out = x1 + gb * y
    o_ref[0] = out[0:1].astype(o_ref.dtype)


@jax.jit
def pallas_adaLN_cond__sliding_block_cached__geglu_ffn__decode_kernel(
    A_x: jax.Array,
    A_k_cache: jax.Array,
    A_v_cache: jax.Array,
    A_wq: jax.Array,
    A_wo: jax.Array,
    B_x: jax.Array,
    B_w_gate: jax.Array,
    B_w_up: jax.Array,
    B_w_down: jax.Array,
    c: jax.Array,
    w_mod: jax.Array,
):
    del B_x
    B, Sq, D = A_x.shape
    _, Hkv, Sk, Dh = A_k_cache.shape
    F = B_w_gate.shape[1]
    assert (B, Sq, Hkv, Dh) == (1, 1, _H, _DH)
    window = min(4096, max(256, Sk // 4))

    kt = jnp.swapaxes(A_k_cache, 2, 3).reshape(_H * _DH, Sk)
    vt = jnp.swapaxes(A_v_cache, 2, 3).reshape(_H * _DH, Sk)
    wo = A_wo.reshape(_NP, _PAIR, D)

    bf16 = jnp.bfloat16
    any_spec = pl.BlockSpec(memory_space=pl.ANY)
    return pl.pallas_call(
        functools.partial(_kernel, window=window, d_model=D),
        in_specs=[any_spec] * 10,
        out_specs=pl.BlockSpec(memory_space=pltpu.VMEM),
        out_shape=jax.ShapeDtypeStruct(A_x.shape, A_x.dtype),
        scratch_shapes=[
            pltpu.VMEM(A_x.shape, A_x.dtype),
            pltpu.VMEM(c.shape, c.dtype),
            pltpu.VMEM(w_mod.shape, bf16),
            pltpu.VMEM(A_wq.shape, bf16),
            pltpu.VMEM(wo.shape, bf16),
            pltpu.VMEM(B_w_gate.shape, bf16),
            pltpu.VMEM(B_w_up.shape, bf16),
            pltpu.VMEM(B_w_down.shape, bf16),
            pltpu.VMEM((_NS, _PAIR, window), bf16),
            pltpu.VMEM((_NS, _PAIR, window), bf16),
            pltpu.VMEM((_NP, _R, _PAIR), bf16),
            pltpu.SemaphoreType.DMA((8,)),
            pltpu.SemaphoreType.DMA((2, _NS)),
        ],
        compiler_params=pltpu.CompilerParams(vmem_limit_bytes=100 * 1024 * 1024),
    )(A_x, c, kt, vt, A_wq, wo, B_w_gate, B_w_up, B_w_down, w_mod)
```

```python
import functools
import math

import jax
import jax.numpy as jnp
import jax.experimental.pallas as pl
import jax.experimental.pallas.tpu as pltpu

_H = 32
_DH = 192
_PAIR = 2 * _DH
_NP = _H // 2
_R = 8
_EPS = 1e-5
_LOG2E = math.log2(math.e)
_NT = (((1,), (1,)), ((), ()))

CFG = dict(
    NS=2,
    KV=(1, 1, 48, 512, 'csr'),
    WM=(8, 4, 8, 640), WQ=(8, 4, 8, 512), WO=(16, 4, 8, 640), WG=(4, 4, 8, 768), WD=(2, 1, 32, 640),
    NWD=3,
    FFN1=80,
    NOBC=False, NOSC=False,
    NOCOMP=0,
)


def _layernorm(x):
    m = jnp.mean(x, axis=-1, keepdims=True)
    d = x - m
    v = jnp.mean(d * d, axis=-1, keepdims=True)
    return d * jax.lax.rsqrt(v + _EPS)


def _dot(a, b):
    return jnp.dot(a, b, preferred_element_type=jnp.float32)


def _tiles(r0, r1, cols, pr, pc, order='rc'):
    rs = list(range(r0, r1, pr)); cs = list(range(0, cols, pc))
    if order == 'rc':
        return [(r, min(pr, r1 - r), c, min(pc, cols - c)) for r in rs for c in cs]
    return [(r, min(pr, r1 - r), c, min(pc, cols - c)) for c in cs for r in rs]


def _kv_pieces(window, n, m, pr, pc, order):
    rn = _PAIR // n
    axes = {'s': list(range(0, n, m)), 'r': list(range(0, rn, pr)), 'c': list(range(0, window, pc))}
    out = []
    for a in axes[order[0]]:
        for b in axes[order[1]]:
            for c_ in axes[order[2]]:
                d = dict(zip(order, (a, b, c_)))
                out.append((d['s'], min(m, n - d['s']), d['r'], min(pr, rn - d['r']), d['c'], min(pc, window - d['c'])))
    return out


def _zip2(a, b):
    out = []
    for i in range(max(len(a), len(b))):
        if i < len(a): out.append(a[i])
        if i < len(b): out.append(b[i])
    return out


def _flat(v):
    return v.reshape(v.shape[0] * v.shape[1], v.shape[2])


def _kernel(x_hbm, c_hbm, k_hbm, v_hbm, wq_hbm, wo_hbm, wg_hbm, wu_hbm, wd_hbm, wm_hbm,
            o_ref,
            x_buf, c_buf, wm_buf, wq_buf, wo_buf, wg_buf, wu_buf, wd_buf, k_buf, v_buf, q_scr,
            w_sem, wd_sem, kv_sem, *, window, d_model, cfg):
    f32, bf16 = jnp.float32, jnp.bfloat16
    sk = k_hbm.shape[3]
    D = d_model
    NS = cfg['NS']
    F = wg_hbm.shape[2]
    NWD = cfg['NWD']

    def wait_all(dst, sem):
        pltpu.make_async_copy(dst, dst, sem).wait()

    def start_list(lst):
        for c_, prio in lst:
            c_.start(priority=prio)

    def slab_pieces(src, dst, sem, s0, s1, spec, r0=0, r1=None):
        n, m, pr, pc = spec
        _, rows, cols = src.shape
        r1 = rows if r1 is None else r1
        return [pltpu.make_async_copy(src.at[s:min(s + m, s1), pl.ds(r, nr), pl.ds(c, nc)],
                                      dst.at[s:min(s + m, s1), pl.ds(r, nr), pl.ds(c, nc)], sem)
                for (r, nr, c, nc) in _tiles(r0, r1, cols, pr, pc) for s in range(s0, s1, m)]

    def halves(src, dst, sem, spec, r0=0, r1=None):
        n = src.shape[0]
        top = [(c_, 0) for c_ in slab_pieces(src, dst, sem, 0, n // 2, spec, r0, r1)]
        bot = [(c_, 1) for c_ in slab_pieces(src, dst, sem, n // 2, n, spec, r0, r1)]
        return _zip2(top, bot)

    def kv_start(p, slot):
        def cp(src, dst, sem, t):
            s0, ms, r, nr, c, nc = t
            return pltpu.make_async_copy(src.at[p, s0:s0 + ms, pl.ds(r, nr), pl.ds(sk - window + c, nc)],
                                         dst.at[s0:s0 + ms, pl.ds(r, nr), pl.ds(c, nc)], sem)
        ts = _kv_pieces(window, *cfg['KV'])
        k = [(cp(k_hbm, k_buf.at[slot], kv_sem.at[0, slot], t), 0) for t in ts]
        v = [(cp(v_hbm, v_buf.at[slot], kv_sem.at[1, slot], t), 1) for t in ts]
        start_list(_zip2(k, v))

    ng = wg_hbm.shape[0]
    g_l = [(c_, 0) for c_ in slab_pieces(wg_hbm, wg_buf, w_sem.at[5], 0, ng, cfg['WG'])]
    u_l = [(c_, 1) for c_ in slab_pieces(wu_hbm, wu_buf, w_sem.at[6], 0, ng, cfg['WG'])]
    hrows = F // 2 // NWD
    d_l = []
    for i in range(NWD):
        d_l += halves(wd_hbm, wd_buf, wd_sem.at[i], cfg['WD'], i * hrows, (i + 1) * hrows)
    ffn_l = _zip2(g_l, u_l) + d_l

    def wd_wait(i):
        wait_all(wd_buf.at[:, pl.ds(i * hrows, hrows), :], wd_sem.at[i])

    c_cp = pltpu.make_async_copy(c_hbm, c_buf, w_sem.at[0])
    x_cp = pltpu.make_async_copy(x_hbm, x_buf, w_sem.at[1])

    def prologue_a():
        c_cp.start()
        x_cp.start()
        start_list(halves(wm_hbm, wm_buf, w_sem.at[2], cfg['WM']))
        start_list(halves(wq_hbm, wq_buf, w_sem.at[3], cfg['WQ']))

    def prologue_b():
        start_list(halves(wo_hbm, wo_buf, w_sem.at[4], cfg['WO']))

    def prologue_c():
        for p in range(NS):
            kv_start(p, p)

    def next_issue(p, slot):
        @pl.when(p + NS < _NP)
        def _():
            kv_start(p + NS, slot)

        @pl.when(p == _NP - 2)
        def _():
            start_list(ffn_l[:cfg['FFN1']])

    def last_issue():
        start_list(ffn_l[cfg['FFN1']:])

    if cfg['NOCOMP']:
        prologue_a()
        c_cp.wait(); x_cp.wait(); wait_all(wm_buf, w_sem.at[2])
        prologue_b()
        wait_all(wq_buf, w_sem.at[3])
        prologue_c()
        wait_all(wo_buf, w_sem.at[4])
        def dummy_step(p, acc):
            slot = p % NS
            wait_all(k_buf.at[slot], kv_sem.at[0, slot])
            wait_all(v_buf.at[slot], kv_sem.at[1, slot])
            if cfg['NOCOMP'] > 1:
                pl.delay(cfg['NOCOMP'])
            next_issue(p, slot)
            return acc
        acc = jax.lax.fori_loop(0, _NP, dummy_step, jnp.zeros((_R, D), f32))
        last_issue()
        wait_all(wg_buf, w_sem.at[5]); wait_all(wu_buf, w_sem.at[6])
        for i in range(NWD):
            wd_wait(i)
        o_ref[0] = acc[0:1].astype(o_ref.dtype)
        return

    prologue_a()

    c_cp.wait()
    c = jnp.broadcast_to(c_buf[...].astype(f32), (_R, D))
    silu_c = (c * jax.nn.sigmoid(c)).astype(bf16)
    wait_all(wm_buf, w_sem.at[2])
    mod = _dot(silu_c, _flat(wm_buf[...]))
    sa, ca, ga, sb, cb, gb = (mod[:, i * D:(i + 1) * D] for i in range(6))

    x_cp.wait()
    x = jnp.broadcast_to(x_buf[0].astype(f32), (_R, D))
    h = (_layernorm(x) * (1.0 + ca) + sa).astype(bf16)

    prologue_b()
    wait_all(wq_buf, w_sem.at[3])
    row = jax.lax.broadcasted_iota(jnp.int32, (_R, _PAIR), 0)
    col = jax.lax.broadcasted_iota(jnp.int32, (_R, _PAIR), 1)
    diag = (col >= row * _DH) & (col < (row + 1) * _DH)
    for p in range(_NP):
        q = _dot(h, _flat(wq_buf[:, :, p * _PAIR:(p + 1) * _PAIR]))
        q_scr[p] = jnp.where(diag, q, 0.0).astype(bf16)

    prologue_c()
    wait_all(wo_buf, w_sem.at[4])
    scale_log2 = (_DH ** -0.5) * _LOG2E
    ppo = wo_buf.shape[1] // _PAIR

    def pair_step(p, acc):
        slot = p % NS
        wait_all(k_buf.at[slot], kv_sem.at[0, slot])
        s = _dot(q_scr[p], _flat(k_buf[slot]))
        m = jnp.max(s, axis=-1, keepdims=True)
        e = jnp.exp2((s - m) * scale_log2)
        l = jnp.sum(e, axis=-1, keepdims=True)
        wait_all(v_buf.at[slot], kv_sem.at[1, slot])
        o = jax.lax.dot_general(e.astype(bf16), _flat(v_buf[slot]), _NT, preferred_element_type=f32)
        o = jnp.where(diag, o / l, 0.0).astype(bf16)
        wo_p = wo_buf[p // ppo, pl.ds(pl.multiple_of((p % ppo) * _PAIR, 128), _PAIR), :]
        acc = acc + _dot(o, wo_p)
        next_issue(p, slot)
        return acc

    attn = jax.lax.fori_loop(0, _NP, pair_step, jnp.zeros((_R, D), f32))
    last_issue()
    attn = jnp.sum(attn, axis=0, keepdims=True)
    x1 = x + ga * attn

    h2 = (_layernorm(x1) * (1.0 + cb) + sb).astype(bf16)
    wait_all(wg_buf, w_sem.at[5])
    g = _dot(h2, _flat(wg_buf[...]))
    wait_all(wu_buf, w_sem.at[6])
    u = _dot(h2, _flat(wu_buf[...]))
    a = (jax.nn.gelu(g, approximate=True) * u).astype(bf16)
    y = jnp.zeros((_R, D), f32)
    for i in range(NWD):
        wd_wait(i)
        for hh in range(2):
            r0 = hh * (F // 2) + i * hrows
            y = y + _dot(a[:, r0:r0 + hrows], wd_buf[hh, i * hrows:(i + 1) * hrows, :])
    out = x1 + gb * y
    o_ref[0] = out[0:1].astype(o_ref.dtype)


def make_kernel(cfg):
    @jax.jit
    def kern(A_x, A_k_cache, A_v_cache, A_wq, A_wo, B_x, B_w_gate, B_w_up, B_w_down, c, w_mod):
        del B_x
        B, Sq, D = A_x.shape
        _, Hkv, Sk, Dh = A_k_cache.shape
        assert (B, Sq, Hkv, Dh) == (1, 1, _H, _DH)
        window = min(4096, max(256, Sk // 4))
        nkv = cfg['KV'][0]
        kt = jnp.swapaxes(A_k_cache, 2, 3).reshape(_NP, nkv, _PAIR // nkv, Sk)
        vt = jnp.swapaxes(A_v_cache, 2, 3).reshape(_NP, nkv, _PAIR // nkv, Sk)
        bf16 = jnp.bfloat16
        NS = cfg['NS']
        slabs = lambda w, n: w.reshape(n, w.shape[0] // n, w.shape[1])
        wm = slabs(w_mod, cfg['WM'][0]); wq = slabs(A_wq, cfg['WQ'][0]); wo = slabs(A_wo, cfg['WO'][0])
        wg = slabs(B_w_gate, cfg['WG'][0]); wu = slabs(B_w_up, cfg['WG'][0]); wd = slabs(B_w_down, cfg['WD'][0])
        any_spec = pl.BlockSpec(memory_space=pl.ANY)
        return pl.pallas_call(
            functools.partial(_kernel, window=window, d_model=D, cfg=cfg),
            in_specs=[any_spec] * 10,
            out_specs=pl.BlockSpec(memory_space=pltpu.VMEM),
            out_shape=jax.ShapeDtypeStruct(A_x.shape, A_x.dtype),
            scratch_shapes=[
                pltpu.VMEM(A_x.shape, A_x.dtype),
                pltpu.VMEM(c.shape, c.dtype),
                pltpu.VMEM(wm.shape, bf16),
                pltpu.VMEM(wq.shape, bf16),
                pltpu.VMEM(wo.shape, bf16),
                pltpu.VMEM(wg.shape, bf16),
                pltpu.VMEM(wu.shape, bf16),
                pltpu.VMEM(wd.shape, bf16),
                pltpu.VMEM((NS, nkv, _PAIR // nkv, window), bf16),
                pltpu.VMEM((NS, nkv, _PAIR // nkv, window), bf16),
                pltpu.VMEM((_NP, _R, _PAIR), bf16),
                pltpu.SemaphoreType.DMA((8,)),
                pltpu.SemaphoreType.DMA((cfg['NWD'],)),
                pltpu.SemaphoreType.DMA((2, NS)),
            ],
            compiler_params=pltpu.CompilerParams(vmem_limit_bytes=100 * 1024 * 1024, disable_bounds_checks=cfg['NOBC'],
                                                 disable_semaphore_checks=cfg['NOSC']),
        )(A_x, c, kt, vt, wq, wo, wg, wu, wd, wm)
    return kern


pallas_adaLN_cond__sliding_block_cached__geglu_ffn__decode_kernel = make_kernel(CFG)
```

```python
import functools
import math

import jax
import jax.numpy as jnp
import jax.experimental.pallas as pl
import jax.experimental.pallas.tpu as pltpu

_H = 32
_DH = 192
_PAIR = 2 * _DH
_NP = _H // 2
_R = 8
_EPS = 1e-5
_NT = (((1,), (1,)), ((), ()))

_KV_PIECE = (128, 128)
_WM = (8, 4, 8, 640)
_WQ = (8, 4, 8, 512)
_WO = (16, 4, 8, 640)
_WGU = (4, 4, 8, 768)
_WD = (2, 1, 32, 640)
_WD_CHUNKS = (384, 256, 128)

_S_CX, _S_WM, _S_WQ, _S_WO, _S_K, _S_V = 0, 1, 2, 3, 4, 6
_S_WG, _S_WU, _S_WD = _S_CX, _S_WM, _S_WQ


def _layernorm(x):
    m = jnp.mean(x, axis=-1, keepdims=True)
    d = x - m
    v = jnp.mean(d * d, axis=-1, keepdims=True)
    return d * jax.lax.rsqrt(v + _EPS)


def _dot(a, b):
    return jnp.dot(a, b, preferred_element_type=jnp.float32)


def _flat(v):
    return v.reshape(v.shape[0] * v.shape[1], v.shape[2])


def _interleave(a, b):
    out = []
    for i in range(max(len(a), len(b))):
        out += a[i:i + 1] + b[i:i + 1]
    return out


def _kernel(x_hbm, c_hbm, k_hbm, v_hbm, wq_hbm, wo_hbm, wg_hbm, wu_hbm, wd_hbm, wm_hbm,
            o_ref,
            x_buf, c_buf, wm_buf, wq_buf, wo_buf, wg_buf, wu_buf, wd_buf, k_buf, v_buf, q_buf,
            sem, *, window):
    f32, bf16 = jnp.float32, jnp.bfloat16
    d_model = x_buf.shape[-1]
    d_ff = wg_hbm.shape[-1]
    sk = k_hbm.shape[-1]

    def wait_all(dst, s):
        pltpu.make_async_copy(dst, dst, sem.at[s]).wait()

    def start(copies):
        for cp, prio in copies:
            cp.start(priority=prio)

    def pieces(src, dst, s, slab0, slab1, spec, prio, row0=0, row1=None):
        _, m, pr, pc = spec
        _, rows, cols = src.shape
        row1 = rows if row1 is None else row1
        out = []
        for r in range(row0, row1, pr):
            for c in range(0, cols, pc):
                for sl in range(slab0, slab1, m):
                    idx = (slice(sl, min(sl + m, slab1)), pl.ds(r, min(pr, row1 - r)), pl.ds(c, min(pc, cols - c)))
                    out.append((pltpu.make_async_copy(src.at[idx], dst.at[idx], sem.at[s]), prio))
        return out

    def both_queues(src, dst, s, spec, row0=0, row1=None):
        n = src.shape[0]
        return _interleave(pieces(src, dst, s, 0, n // 2, spec, 0, row0, row1),
                           pieces(src, dst, s, n // 2, n, spec, 1, row0, row1))

    def kv_start(p, slot):
        pr, pc = _KV_PIECE
        copies = []
        for r in range(0, _PAIR, pr):
            for c in range(0, window, pc):
                for src, dst, s, prio in ((k_hbm, k_buf, _S_K, 0), (v_hbm, v_buf, _S_V, 1)):
                    cp = pltpu.make_async_copy(
                        src.at[p, pl.ds(r, pr), pl.ds(sk - window + c, pc)],
                        dst.at[slot, pl.ds(r, pr), pl.ds(c, pc)], sem.at[s + slot])
                    copies.append((cp, prio))
        start(copies)

    def gate_up_start():
        start(_interleave(pieces(wg_hbm, wg_buf, _S_WG, 0, wg_hbm.shape[0], _WGU, 0),
                          pieces(wu_hbm, wu_buf, _S_WU, 0, wu_hbm.shape[0], _WGU, 1)))

    wd_rows = [(sum(_WD_CHUNKS[:i]), n) for i, n in enumerate(_WD_CHUNKS)]

    def down_start():
        for i, (r0, n) in enumerate(wd_rows):
            start(both_queues(wd_hbm, wd_buf, _S_WD + i, _WD, r0, r0 + n))

    c_copy = pltpu.make_async_copy(c_hbm, c_buf, sem.at[_S_CX])
    x_copy = pltpu.make_async_copy(x_hbm, x_buf, sem.at[_S_CX])

    c_copy.start()
    x_copy.start()
    start(both_queues(wm_hbm, wm_buf, _S_WM, _WM))
    start(both_queues(wq_hbm, wq_buf, _S_WQ, _WQ))

    c_copy.wait()
    x_copy.wait()
    wait_all(wm_buf, _S_WM)
    c = jnp.broadcast_to(c_buf[...].astype(f32), (_R, d_model))
    x = jnp.broadcast_to(x_buf[0].astype(f32), (_R, d_model))
    mod = _dot((c * jax.nn.sigmoid(c)).astype(bf16), _flat(wm_buf[...]))
    sa, ca, ga, sb, cb, gb = (mod[:, i * d_model:(i + 1) * d_model] for i in range(6))
    h = (_layernorm(x) * (1.0 + ca) + sa).astype(bf16)

    start(both_queues(wo_hbm, wo_buf, _S_WO, _WO))
    wait_all(wq_buf, _S_WQ)
    row = jax.lax.broadcasted_iota(jnp.int32, (_R, _PAIR), 0)
    col = jax.lax.broadcasted_iota(jnp.int32, (_R, _PAIR), 1)
    diag = (col >= row * _DH) & (col < (row + 1) * _DH)
    for p in range(_NP):
        q = _dot(h, _flat(wq_buf[:, :, p * _PAIR:(p + 1) * _PAIR]))
        q_buf[p] = jnp.where(diag, q, 0.0).astype(bf16)

    kv_start(0, 0)
    kv_start(1, 1)
    wait_all(wo_buf, _S_WO)
    scale_log2e = _DH ** -0.5 * math.log2(math.e)
    pairs_per_slab = wo_buf.shape[1] // _PAIR

    def pair_step(p, acc):
        slot = p % 2
        wait_all(k_buf.at[slot], _S_K + slot)
        s = _dot(q_buf[p], k_buf[slot])
        m = jnp.max(s, axis=-1, keepdims=True)
        e = jnp.exp2((s - m) * scale_log2e)
        l = jnp.sum(e, axis=-1, keepdims=True)
        wait_all(v_buf.at[slot], _S_V + slot)
        o = jax.lax.dot_general(e.astype(bf16), v_buf[slot], _NT, preferred_element_type=f32)
        o = jnp.where(diag, o / l, 0.0).astype(bf16)
        wo_p = wo_buf[p // pairs_per_slab,
                      pl.ds(pl.multiple_of((p % pairs_per_slab) * _PAIR, 128), _PAIR), :]
        acc = acc + _dot(o, wo_p)

        @pl.when(p + 2 < _NP)
        def _():
            kv_start(p + 2, slot)

        @pl.when(p + 2 == _NP)
        def _():
            gate_up_start()

        return acc

    attn = jax.lax.fori_loop(0, _NP, pair_step, jnp.zeros((_R, d_model), f32))
    down_start()
    x = x + ga * jnp.sum(attn, axis=0, keepdims=True)

    h = (_layernorm(x) * (1.0 + cb) + sb).astype(bf16)
    wait_all(wg_buf, _S_WG)
    g = _dot(h, _flat(wg_buf[...]))
    wait_all(wu_buf, _S_WU)
    u = _dot(h, _flat(wu_buf[...]))
    a = (jax.nn.gelu(g, approximate=True) * u).astype(bf16)
    y = jnp.zeros((_R, d_model), f32)
    for i, (r0, n) in enumerate(wd_rows):
        wait_all(wd_buf.at[:, pl.ds(r0, n), :], _S_WD + i)
        for half in range(2):
            f0 = half * (d_ff // 2) + r0
            y = y + _dot(a[:, f0:f0 + n], wd_buf[half, r0:r0 + n, :])
    o_ref[0] = (x + gb * y)[0:1].astype(o_ref.dtype)


@jax.jit
def pallas_adaLN_cond__sliding_block_cached__geglu_ffn__decode_kernel(
    A_x: jax.Array,
    A_k_cache: jax.Array,
    A_v_cache: jax.Array,
    A_wq: jax.Array,
    A_wo: jax.Array,
    B_x: jax.Array,
    B_w_gate: jax.Array,
    B_w_up: jax.Array,
    B_w_down: jax.Array,
    c: jax.Array,
    w_mod: jax.Array,
):
    del B_x
    B, Sq, D = A_x.shape
    _, Hkv, Sk, Dh = A_k_cache.shape
    F = B_w_gate.shape[1]
    assert (B, Sq, Hkv, Dh) == (1, 1, _H, _DH) and sum(_WD_CHUNKS) * 2 == F
    window = min(4096, max(256, Sk // 4))

    kt = jnp.swapaxes(A_k_cache, 2, 3).reshape(_NP, _PAIR, Sk)
    vt = jnp.swapaxes(A_v_cache, 2, 3).reshape(_NP, _PAIR, Sk)
    slabs = lambda w, spec: w.reshape(spec[0], w.shape[0] // spec[0], w.shape[1])
    wm, wq, wo = slabs(w_mod, _WM), slabs(A_wq, _WQ), slabs(A_wo, _WO)
    wg, wu, wd = slabs(B_w_gate, _WGU), slabs(B_w_up, _WGU), slabs(B_w_down, _WD)

    vmem = lambda a: pltpu.VMEM(a.shape, a.dtype)
    return pl.pallas_call(
        functools.partial(_kernel, window=window),
        in_specs=[pl.BlockSpec(memory_space=pl.ANY)] * 10,
        out_specs=pl.BlockSpec(memory_space=pltpu.VMEM),
        out_shape=jax.ShapeDtypeStruct(A_x.shape, A_x.dtype),
        scratch_shapes=[
            vmem(A_x), vmem(c), vmem(wm), vmem(wq), vmem(wo), vmem(wg), vmem(wu), vmem(wd),
            pltpu.VMEM((2, _PAIR, window), kt.dtype),
            pltpu.VMEM((2, _PAIR, window), vt.dtype),
            pltpu.VMEM((_NP, _R, _PAIR), jnp.bfloat16),
            pltpu.SemaphoreType.DMA((8,)),
        ],
        compiler_params=pltpu.CompilerParams(vmem_limit_bytes=100 * 1024 * 1024),
    )(A_x, c, kt, vt, wq, wo, wg, wu, wd, wm)
```

```python
import functools
import math

import jax
import jax.numpy as jnp
import jax.experimental.pallas as pl
import jax.experimental.pallas.tpu as pltpu

_H = 32
_DH = 192
_PAIR = 2 * _DH
_NP = _H // 2
_R = 8
_EPS = 1e-5
_NT = (((1,), (1,)), ((), ()))

_KV_PIECE = (128, 128)
_WM = (8, 4, 8, 640)
_WQ = (8, 4, 8, 512)
_WO = (_NP, 4, 8, 640)
_WGU = (4, 4, 8, 768)
_WD = (2, 1, 32, 640)
_WD_CHUNKS = (384, 256, 128)

_S_CX, _S_WM, _S_WQ, _S_WO, _S_K, _S_V = 0, 1, 2, 3, 4, 6
_S_WG, _S_WU, _S_WD = _S_CX, _S_WM, _S_WQ


def _layernorm(x):
    m = jnp.mean(x, axis=-1, keepdims=True)
    d = x - m
    v = jnp.mean(d * d, axis=-1, keepdims=True)
    return d * jax.lax.rsqrt(v + _EPS)


def _dot(a, b):
    return jnp.dot(a, b, preferred_element_type=jnp.float32)


def _flat(v):
    return v.reshape(v.shape[0] * v.shape[1], v.shape[2])


def _interleave(a, b):
    out = []
    for i in range(max(len(a), len(b))):
        out += a[i:i + 1] + b[i:i + 1]
    return out


def _kernel(x_hbm, c_hbm, k_hbm, v_hbm, wq_hbm, wo_hbm, wg_hbm, wu_hbm, wd_hbm, wm_hbm,
            o_ref,
            x_buf, c_buf, wm_buf, wq_buf, wo_buf, wg_buf, wu_buf, wd_buf, k_buf, v_buf, q_buf,
            sem, *, window):
    f32, bf16 = jnp.float32, jnp.bfloat16
    d_model = x_buf.shape[-1]
    d_ff = wg_hbm.shape[-1]
    sk = k_hbm.shape[-1]

    def wait_all(dst, s):
        pltpu.make_async_copy(dst, dst, sem.at[s]).wait()

    def start(copies):
        for cp, prio in copies:
            cp.start(priority=prio)

    def pieces(src, dst, s, slab0, slab1, spec, prio, row0=0, row1=None):
        _, m, pr, pc = spec
        _, rows, cols = src.shape
        row1 = rows if row1 is None else row1
        out = []
        for r in range(row0, row1, pr):
            for c in range(0, cols, pc):
                for sl in range(slab0, slab1, m):
                    idx = (slice(sl, min(sl + m, slab1)), pl.ds(r, min(pr, row1 - r)), pl.ds(c, min(pc, cols - c)))
                    out.append((pltpu.make_async_copy(src.at[idx], dst.at[idx], sem.at[s]), prio))
        return out

    def both_queues(src, dst, s, spec, row0=0, row1=None):
        n = src.shape[0]
        return _interleave(pieces(src, dst, s, 0, n // 2, spec, 0, row0, row1),
                           pieces(src, dst, s, n // 2, n, spec, 1, row0, row1))

    def kv_start(p, slot):
        pr, pc = _KV_PIECE
        copies = []
        for r in range(0, _PAIR, pr):
            for c in range(0, window, pc):
                for src, dst, s, prio in ((k_hbm, k_buf, _S_K, 0), (v_hbm, v_buf, _S_V, 1)):
                    cp = pltpu.make_async_copy(
                        src.at[p, pl.ds(r, pr), pl.ds(sk - window + c, pc)],
                        dst.at[slot, pl.ds(r, pr), pl.ds(c, pc)], sem.at[s + slot])
                    copies.append((cp, prio))
        start(copies)

    def gate_up_start():
        start(_interleave(pieces(wg_hbm, wg_buf, _S_WG, 0, wg_hbm.shape[0], _WGU, 0),
                          pieces(wu_hbm, wu_buf, _S_WU, 0, wu_hbm.shape[0], _WGU, 1)))

    wd_rows = [(sum(_WD_CHUNKS[:i]), n) for i, n in enumerate(_WD_CHUNKS)]

    def down_start():
        for i, (r0, n) in enumerate(wd_rows):
            start(both_queues(wd_hbm, wd_buf, _S_WD + i, _WD, r0, r0 + n))

    c_copy = pltpu.make_async_copy(c_hbm, c_buf, sem.at[_S_CX])
    x_copy = pltpu.make_async_copy(x_hbm, x_buf, sem.at[_S_CX])

    c_copy.start()
    x_copy.start()
    start(both_queues(wm_hbm, wm_buf, _S_WM, _WM))
    start(both_queues(wq_hbm, wq_buf, _S_WQ, _WQ))

    c_copy.wait()
    x_copy.wait()
    wait_all(wm_buf, _S_WM)
    c = jnp.broadcast_to(c_buf[...].astype(f32), (_R, d_model))
    x = jnp.broadcast_to(x_buf[0].astype(f32), (_R, d_model))
    mod = _dot((c * jax.nn.sigmoid(c)).astype(bf16), _flat(wm_buf[...]))
    sa, ca, ga, sb, cb, gb = (mod[:, i * d_model:(i + 1) * d_model] for i in range(6))
    h = (_layernorm(x) * (1.0 + ca) + sa).astype(bf16)

    start(both_queues(wo_hbm, wo_buf, _S_WO, _WO))
    wait_all(wq_buf, _S_WQ)
    row = jax.lax.broadcasted_iota(jnp.int32, (_R, _PAIR), 0)
    col = jax.lax.broadcasted_iota(jnp.int32, (_R, _PAIR), 1)
    diag = (col >= row * _DH) & (col < (row + 1) * _DH)
    for p in range(_NP):
        q = _dot(h, _flat(wq_buf[:, :, p * _PAIR:(p + 1) * _PAIR]))
        q_buf[p] = jnp.where(diag, q, 0.0).astype(bf16)

    kv_start(0, 0)
    kv_start(1, 1)
    wait_all(wo_buf, _S_WO)
    scale_log2e = _DH ** -0.5 * math.log2(math.e)

    def pair_step(p, acc):
        slot = p % 2
        wait_all(k_buf.at[slot], _S_K + slot)
        s = _dot(q_buf[p], k_buf[slot])
        m = jnp.max(s, axis=-1, keepdims=True)
        e = jnp.exp2((s - m) * scale_log2e)
        l = jnp.sum(e, axis=-1, keepdims=True)
        wait_all(v_buf.at[slot], _S_V + slot)
        o = jax.lax.dot_general(e.astype(bf16), v_buf[slot], _NT, preferred_element_type=f32)
        o = jnp.where(diag, o / l, 0.0).astype(bf16)
        acc = acc + _dot(o, wo_buf[p])

        @pl.when(p + 2 < _NP)
        def _():
            kv_start(p + 2, slot)

        @pl.when(p + 2 == _NP)
        def _():
            gate_up_start()

        return acc

    attn = jax.lax.fori_loop(0, _NP, pair_step, jnp.zeros((_R, d_model), f32))
    down_start()
    x = x + ga * jnp.sum(attn, axis=0, keepdims=True)

    h = (_layernorm(x) * (1.0 + cb) + sb).astype(bf16)
    wait_all(wg_buf, _S_WG)
    g = _dot(h, _flat(wg_buf[...]))
    wait_all(wu_buf, _S_WU)
    u = _dot(h, _flat(wu_buf[...]))
    a = (jax.nn.gelu(g, approximate=True) * u).astype(bf16)
    y = jnp.zeros((_R, d_model), f32)
    for i, (r0, n) in enumerate(wd_rows):
        wait_all(wd_buf.at[:, pl.ds(r0, n), :], _S_WD + i)
        for half in range(2):
            f0 = half * (d_ff // 2) + r0
            y = y + _dot(a[:, f0:f0 + n], wd_buf[half, r0:r0 + n, :])
    o_ref[0] = (x + gb * y)[0:1].astype(o_ref.dtype)


@jax.jit
def pallas_adaLN_cond__sliding_block_cached__geglu_ffn__decode_kernel(
    A_x: jax.Array,
    A_k_cache: jax.Array,
    A_v_cache: jax.Array,
    A_wq: jax.Array,
    A_wo: jax.Array,
    B_x: jax.Array,
    B_w_gate: jax.Array,
    B_w_up: jax.Array,
    B_w_down: jax.Array,
    c: jax.Array,
    w_mod: jax.Array,
):
    del B_x
    B, Sq, D = A_x.shape
    _, Hkv, Sk, Dh = A_k_cache.shape
    F = B_w_gate.shape[1]
    assert (B, Sq, Hkv, Dh) == (1, 1, _H, _DH) and sum(_WD_CHUNKS) * 2 == F
    window = min(4096, max(256, Sk // 4))

    kt = jnp.swapaxes(A_k_cache, 2, 3).reshape(_NP, _PAIR, Sk)
    vt = jnp.swapaxes(A_v_cache, 2, 3).reshape(_NP, _PAIR, Sk)
    slabs = lambda w, spec: w.reshape(spec[0], w.shape[0] // spec[0], w.shape[1])
    wm, wq, wo = slabs(w_mod, _WM), slabs(A_wq, _WQ), slabs(A_wo, _WO)
    wg, wu, wd = slabs(B_w_gate, _WGU), slabs(B_w_up, _WGU), slabs(B_w_down, _WD)

    vmem = lambda a: pltpu.VMEM(a.shape, a.dtype)
    return pl.pallas_call(
        functools.partial(_kernel, window=window),
        in_specs=[pl.BlockSpec(memory_space=pl.ANY)] * 10,
        out_specs=pl.BlockSpec(memory_space=pltpu.VMEM),
        out_shape=jax.ShapeDtypeStruct(A_x.shape, A_x.dtype),
        scratch_shapes=[
            vmem(A_x), vmem(c), vmem(wm), vmem(wq), vmem(wo), vmem(wg), vmem(wu), vmem(wd),
            pltpu.VMEM((2, _PAIR, window), kt.dtype),
            pltpu.VMEM((2, _PAIR, window), vt.dtype),
            pltpu.VMEM((_NP, _R, _PAIR), jnp.bfloat16),
            pltpu.SemaphoreType.DMA((8,)),
        ],
        compiler_params=pltpu.CompilerParams(vmem_limit_bytes=100 * 1024 * 1024),
    )(A_x, c, kt, vt, wq, wo, wg, wu, wd, wm)
```

```python
import functools
import math

import jax
import jax.numpy as jnp
import jax.experimental.pallas as pl
import jax.experimental.pallas.tpu as pltpu

_H = 32
_DH = 192
_PAIR = 2 * _DH
_NP = _H // 2
_R = 8
_EPS = 1e-5
_NT = (((1,), (1,)), ((), ()))

_K_PIECE = (128, 128)
_V_PIECE = (64, 256)
_WM = (8, 4, 8, 640)
_WQ = (8, 4, 8, 512)
_WO = (_NP, 4, 8, 640)
_WGU = (4, 4, 8, 768)
_WD = (2, 1, 32, 640)
_WD_CHUNKS = (384, 256, 128)

_S_CX, _S_WM, _S_WQ, _S_WO, _S_K, _S_V = 0, 1, 2, 3, 4, 6
_S_WG, _S_WU, _S_WD = _S_CX, _S_WM, _S_WQ


def _layernorm(x):
    m = jnp.mean(x, axis=-1, keepdims=True)
    d = x - m
    v = jnp.mean(d * d, axis=-1, keepdims=True)
    return d * jax.lax.rsqrt(v + _EPS)


def _dot(a, b):
    return jnp.dot(a, b, preferred_element_type=jnp.float32)


def _flat(v):
    return v.reshape(v.shape[0] * v.shape[1], v.shape[2])


def _interleave(a, b):
    out = []
    for i in range(max(len(a), len(b))):
        out += a[i:i + 1] + b[i:i + 1]
    return out


def _kernel(x_hbm, c_hbm, k_hbm, v_hbm, wq_hbm, wo_hbm, wg_hbm, wu_hbm, wd_hbm, wm_hbm,
            o_ref,
            x_buf, c_buf, wm_buf, wq_buf, wo_buf, wg_buf, wu_buf, wd_buf, k_buf, v_buf, q_buf,
            sem, *, window):
    f32, bf16 = jnp.float32, jnp.bfloat16
    d_model = x_buf.shape[-1]
    d_ff = wg_hbm.shape[-1]
    sk = k_hbm.shape[-1]

    def wait_all(dst, s):
        pltpu.make_async_copy(dst, dst, sem.at[s]).wait()

    def start(copies):
        for cp, prio in copies:
            cp.start(priority=prio)

    def pieces(src, dst, s, slab0, slab1, spec, prio, row0=0, row1=None):
        _, m, pr, pc = spec
        _, rows, cols = src.shape
        row1 = rows if row1 is None else row1
        out = []
        for r in range(row0, row1, pr):
            for c in range(0, cols, pc):
                for sl in range(slab0, slab1, m):
                    idx = (slice(sl, min(sl + m, slab1)), pl.ds(r, min(pr, row1 - r)), pl.ds(c, min(pc, cols - c)))
                    out.append((pltpu.make_async_copy(src.at[idx], dst.at[idx], sem.at[s]), prio))
        return out

    def both_queues(src, dst, s, spec, row0=0, row1=None):
        n = src.shape[0]
        return _interleave(pieces(src, dst, s, 0, n // 2, spec, 0, row0, row1),
                           pieces(src, dst, s, n // 2, n, spec, 1, row0, row1))

    def kv_start(p, slot):
        streams = []
        for src, dst, s, prio, (pr, pc) in ((k_hbm, k_buf, _S_K, 0, _K_PIECE), (v_hbm, v_buf, _S_V, 1, _V_PIECE)):
            streams.append([
                (pltpu.make_async_copy(src.at[p, pl.ds(r, pr), pl.ds(sk - window + c, pc)],
                                       dst.at[slot, pl.ds(r, pr), pl.ds(c, pc)], sem.at[s + slot]), prio)
                for r in range(0, _PAIR, pr) for c in range(0, window, pc)])
        start(_interleave(*streams))

    def gate_up_start():
        start(_interleave(pieces(wg_hbm, wg_buf, _S_WG, 0, wg_hbm.shape[0], _WGU, 0),
                          pieces(wu_hbm, wu_buf, _S_WU, 0, wu_hbm.shape[0], _WGU, 1)))

    wd_rows = [(sum(_WD_CHUNKS[:i]), n) for i, n in enumerate(_WD_CHUNKS)]

    def down_start():
        for i, (r0, n) in enumerate(wd_rows):
            start(both_queues(wd_hbm, wd_buf, _S_WD + i, _WD, r0, r0 + n))

    c_copy = pltpu.make_async_copy(c_hbm, c_buf, sem.at[_S_CX])
    x_copy = pltpu.make_async_copy(x_hbm, x_buf, sem.at[_S_CX])

    c_copy.start()
    x_copy.start()
    start(both_queues(wm_hbm, wm_buf, _S_WM, _WM))
    start(both_queues(wq_hbm, wq_buf, _S_WQ, _WQ))

    c_copy.wait()
    x_copy.wait()
    wait_all(wm_buf, _S_WM)
    c = jnp.broadcast_to(c_buf[...].astype(f32), (_R, d_model))
    x = jnp.broadcast_to(x_buf[0].astype(f32), (_R, d_model))
    mod = _dot((c * jax.nn.sigmoid(c)).astype(bf16), _flat(wm_buf[...]))
    sa, ca, ga, sb, cb, gb = (mod[:, i * d_model:(i + 1) * d_model] for i in range(6))
    h = (_layernorm(x) * (1.0 + ca) + sa).astype(bf16)

    start(both_queues(wo_hbm, wo_buf, _S_WO, _WO))
    wait_all(wq_buf, _S_WQ)
    row = jax.lax.broadcasted_iota(jnp.int32, (_R, _PAIR), 0)
    col = jax.lax.broadcasted_iota(jnp.int32, (_R, _PAIR), 1)
    diag = (col >= row * _DH) & (col < (row + 1) * _DH)
    for p in range(_NP):
        q = _dot(h, _flat(wq_buf[:, :, p * _PAIR:(p + 1) * _PAIR]))
        q_buf[p] = jnp.where(diag, q, 0.0).astype(bf16)

    kv_start(0, 0)
    kv_start(1, 1)
    wait_all(wo_buf, _S_WO)
    scale_log2e = _DH ** -0.5 * math.log2(math.e)

    def pair_step(p, acc):
        slot = p % 2
        wait_all(k_buf.at[slot], _S_K + slot)
        s = _dot(q_buf[p], k_buf[slot])
        m = jnp.max(s, axis=-1, keepdims=True)
        e = jnp.exp2((s - m) * scale_log2e)
        l = jnp.sum(e, axis=-1, keepdims=True)
        wait_all(v_buf.at[slot], _S_V + slot)
        o = jax.lax.dot_general(e.astype(bf16), v_buf[slot], _NT, preferred_element_type=f32)
        o = jnp.where(diag, o / l, 0.0).astype(bf16)
        acc = acc + _dot(o, wo_buf[p])

        @pl.when(p + 2 < _NP)
        def _():
            kv_start(p + 2, slot)

        @pl.when(p + 2 == _NP)
        def _():
            gate_up_start()

        return acc

    attn = jax.lax.fori_loop(0, _NP, pair_step, jnp.zeros((_R, d_model), f32))
    down_start()
    x = x + ga * jnp.sum(attn, axis=0, keepdims=True)

    h = (_layernorm(x) * (1.0 + cb) + sb).astype(bf16)
    wait_all(wg_buf, _S_WG)
    g = _dot(h, _flat(wg_buf[...]))
    wait_all(wu_buf, _S_WU)
    u = _dot(h, _flat(wu_buf[...]))
    a = (jax.nn.gelu(g, approximate=True) * u).astype(bf16)
    y = jnp.zeros((_R, d_model), f32)
    for i, (r0, n) in enumerate(wd_rows):
        wait_all(wd_buf.at[:, pl.ds(r0, n), :], _S_WD + i)
        for half in range(2):
            f0 = half * (d_ff // 2) + r0
            y = y + _dot(a[:, f0:f0 + n], wd_buf[half, r0:r0 + n, :])
    o_ref[0] = (x + gb * y)[0:1].astype(o_ref.dtype)


@jax.jit
def pallas_adaLN_cond__sliding_block_cached__geglu_ffn__decode_kernel(
    A_x: jax.Array,
    A_k_cache: jax.Array,
    A_v_cache: jax.Array,
    A_wq: jax.Array,
    A_wo: jax.Array,
    B_x: jax.Array,
    B_w_gate: jax.Array,
    B_w_up: jax.Array,
    B_w_down: jax.Array,
    c: jax.Array,
    w_mod: jax.Array,
):
    del B_x
    B, Sq, D = A_x.shape
    _, Hkv, Sk, Dh = A_k_cache.shape
    F = B_w_gate.shape[1]
    window = min(4096, max(256, Sk // 4))
    assert (B, Sq, Hkv, Dh) == (1, 1, _H, _DH) and sum(_WD_CHUNKS) * 2 == F and window % 256 == 0

    kt = jnp.swapaxes(A_k_cache, 2, 3).reshape(_NP, _PAIR, Sk)
    vt = jnp.swapaxes(A_v_cache, 2, 3).reshape(_NP, _PAIR, Sk)
    slabs = lambda w, spec: w.reshape(spec[0], w.shape[0] // spec[0], w.shape[1])
    wm, wq, wo = slabs(w_mod, _WM), slabs(A_wq, _WQ), slabs(A_wo, _WO)
    wg, wu, wd = slabs(B_w_gate, _WGU), slabs(B_w_up, _WGU), slabs(B_w_down, _WD)

    vmem = lambda a: pltpu.VMEM(a.shape, a.dtype)
    return pl.pallas_call(
        functools.partial(_kernel, window=window),
        in_specs=[pl.BlockSpec(memory_space=pl.ANY)] * 10,
        out_specs=pl.BlockSpec(memory_space=pltpu.VMEM),
        out_shape=jax.ShapeDtypeStruct(A_x.shape, A_x.dtype),
        scratch_shapes=[
            vmem(A_x), vmem(c), vmem(wm), vmem(wq), vmem(wo), vmem(wg), vmem(wu), vmem(wd),
            pltpu.VMEM((2, _PAIR, window), kt.dtype),
            pltpu.VMEM((2, _PAIR, window), vt.dtype),
            pltpu.VMEM((_NP, _R, _PAIR), jnp.bfloat16),
            pltpu.SemaphoreType.DMA((8,)),
        ],
        compiler_params=pltpu.CompilerParams(vmem_limit_bytes=100 * 1024 * 1024),
    )(A_x, c, kt, vt, wq, wo, wg, wu, wd, wm)
```
